```python
import jax
import jax.numpy as jnp

def _softmax(x, axis=-1):
    return jax.nn.softmax(x, axis=axis)
def _gelu(x):
    return jax.nn.gelu(x, approximate=True)
def _silu(x):
    return jax.nn.silu(x)
def _sigmoid(x):
    return jax.nn.sigmoid(x)
def _layernorm(x, axis=-1, eps=1e-5):
    m = jnp.mean(x, axis=axis, keepdims=True)
    v = jnp.var(x, axis=axis, keepdims=True)
    return (x - m) / jnp.sqrt(v + eps)
def _scatter_add(tgt, idx, src, axis=0):
    return tgt.at[idx].add(src)
def _segment_sum(src, seg, n):
    return jax.ops.segment_sum(src, seg, n)
class _Rng:
    def __init__(self, key):
        self._k = key
    def _next(self):
        self._k, sub = jax.random.split(self._k)
        return sub
    def normal(self, shape):
        return jax.random.normal(self._next(), shape, dtype=jnp.bfloat16)
    def randint(self, lo, hi, shape):
        return jax.random.randint(self._next(), shape, lo, hi, dtype=jnp.int32)
    def uniform(self, shape, lo=0.0, hi=1.0):
        return jax.random.uniform(self._next(), shape, jnp.bfloat16, lo, hi)
    def permutation(self, n):
        return jax.random.permutation(self._next(), n)


kernel_name = 'standalone__batchnorm__sampling'

def setup_inputs():
    _rng = _Rng(jax.random.key(int.from_bytes(__import__("os").urandom(4), "little")))
    _w = (lambda a: (lambda t: t.astype(jnp.bfloat16) if jnp.issubdtype(t.dtype, jnp.floating) else t)(jnp.asarray(a)))
    B, S, C = 1024, 32, 576
    K = 3
    return {
        "x": _w((lambda *s: _rng.normal(s) * 0.05)(B, S, C)),
        "w": _w((lambda *s: _rng.normal(s) * 0.05)(K, C, C) * (1.0 / (K * C) ** 0.5)),
        "mean": _w((lambda *s: _rng.normal(s) * 0.05)(C) * 0.1),
        "var": _w(jnp.abs((lambda *s: _rng.normal(s) * 0.05)(C)) + 0.5),
        "g": _w((lambda *s: _rng.normal(s) * 0.05)(C) + 1.0),
        "b": _w((lambda *s: _rng.normal(s) * 0.05)(C) * 0.1),
    }

def reference(x, w, mean, var, g, b):
    K = 3
    P = K // 2
    S = x.shape[1]
    xp = jnp.pad(x, ((0, 0), (P, P), (0, 0)))
    y = sum(jnp.einsum('bsc,cd->bsd', xp[:, k:k + S, :], w[k]) for k in range(K))
    inv_std = 1.0 / jnp.sqrt(var + 1e-5)
    y = (y - mean) * (g * inv_std) + b
    return _silu(y)
```

```python
import numpy as np
import jax
import jax.numpy as jnp
from jax import lax
import jax.experimental.pallas as pl
import jax.experimental.pallas.tpu as pltpu

_A = 1.5
_B = 2.0 / 3.0


def _filter_matrix():
    pts = [0.0, _A, -_A, _B, -_B]
    G = np.zeros((6, 3))
    for i, p in enumerate(pts):
        f = np.prod([p - q for k, q in enumerate(pts) if k != i])
        G[i] = [1.0 / f, p / f, p * p / f]
    G[5] = [0.0, 0.0, 1.0]
    return G


_G = _filter_matrix()


def _input_transform(d):
    d0, d1, d2, d3, d4, d5 = d
    a2, b2 = _A * _A, _B * _B
    a2d2 = a2 * d2
    b2d2 = b2 * d2
    eb = d4 - b2d2
    ea = d4 - a2d2
    ob = _A * (d3 - b2 * d1)
    oa = _B * (d3 - a2 * d1)
    t0 = (ea - b2d2) + d0
    t5 = (d5 + d1) - (a2 + b2) * d3
    return [t0, eb + ob, eb - ob, ea + oa, ea - oa, t5]


def _output_transform(m):
    m0, m1, m2, m3, m4, m5 = m
    s1 = m1 + m2
    d1 = m1 - m2
    s2 = m3 + m4
    d2 = m3 - m4
    y0 = m0 + s1 + s2
    y1 = _A * d1 + _B * d2
    y2 = (_A * _A) * s1 + (_B * _B) * s2
    y3 = (_A ** 3) * d1 + (_B ** 3) * d2 + m5
    return [y0, y1, y2, y3]


def _make_kernel(S, C, B, bn, R, lag1, lag3, n1, n3):
    NG = S // 4
    NI = (B // bn) * NG
    KT = -(-C // 128)
    f32, bf16, u32 = jnp.float32, jnp.bfloat16, jnp.uint32

    def kernel(x_hbm, w_ref, mean_ref, var_ref, g_ref, b_ref, o_hbm,
               xbuf, tbuf, mbuf, obuf, ubuf, bias_ref, xsem, osem):
        def rem(t, m):
            return t % m if isinstance(t, int) else (t & (m - 1))

        def div(t, m):
            if isinstance(t, int):
                return t // m
            return lax.shift_right_logical(t, int(np.log2(m)))

        def window(ref, c):
            return ref.at[pl.ds(rem(c, NG) * 4, 4), :,
                          pl.ds(pl.multiple_of(div(c, NG) * bn, bn), bn)]

        def xcopy(c, slot):
            return pltpu.make_async_copy(window(x_hbm, c), xbuf.at[slot], xsem.at[slot])

        def ocopy(c, slot):
            return pltpu.make_async_copy(obuf.at[slot], window(o_hbm, c), osem.at[slot])

        for c in range(R - 1):
            xcopy(c, c).start()

        def ld(r):
            return r[...].astype(f32)[None, :]

        sc = ld(g_ref) * (1.0 / jnp.sqrt(ld(var_ref) + 1e-5))
        bias = (ld(b_ref) - ld(mean_ref) * sc) * 0.5
        bias_ref[...] = jnp.broadcast_to(bias, (128, C)).T
        sch = sc * 0.5
        wk = [w_ref[k].astype(f32) * sch for k in range(3)]
        ea = _G[1, 0] * wk[0] + _G[1, 2] * wk[2]
        oa = _G[1, 1] * wk[1]
        eb = _G[3, 0] * wk[0] + _G[3, 2] * wk[2]
        ob = _G[3, 1] * wk[1]
        us = [wk[0], ea + oa, ea - oa, eb + ob, eb - ob, wk[2]]
        for i in range(6):
            ut = us[i].astype(bf16).T
            for kk in range(KT):
                wdt = min(128, C - kk * 128)
                if wdt == 128:
                    v = ut[:, kk * 128:(kk + 1) * 128]
                else:
                    v = jnp.concatenate(
                        [ut[:, kk * 128:], jnp.zeros((C, 128 - wdt), bf16)], axis=1)
                ubuf[i, kk] = pltpu.bitcast(v, u32)
        for sl in range(2):
            for i in range(6):
                tbuf[sl, i, C // 2:, :] = jnp.zeros((KT * 64 - C // 2, bn), u32)

        def s1(t, lo=0, hi=C):
            g = rem(t, NG)
            sl = rem(t, 2)
            cm, cc, cp = rem(t + R - 1, R), rem(t, R), rem(t + 1, R)
            rs = pl.ds(lo, hi - lo)
            d0 = jnp.where(g > 0, xbuf[cm, 3, rs, :].astype(f32), 0.0)
            d5 = jnp.where(g < NG - 1, xbuf[cp, 0, rs, :].astype(f32), 0.0)
            d = [d0] + [xbuf[cc, j, rs, :].astype(f32) for j in range(4)] + [d5]
            tt = _input_transform(d)
            for i in range(6):
                tbuf[sl, i, pl.ds(lo // 2, (hi - lo) // 2), :] = pltpu.bitcast(
                    tt[i].astype(bf16), u32)

        def s2(t, i):
            sl = rem(t, 2)
            acc = None
            for kk in range(KT):
                lhs = pltpu.bitcast(ubuf[i, kk], bf16)
                rhs = pltpu.bitcast(tbuf[sl, i, kk * 64:(kk + 1) * 64, :], bf16)
                p = jnp.dot(lhs, rhs, preferred_element_type=f32)
                acc = p if acc is None else acc + p
            mbuf[sl, i] = acc

        def s3(t, lo=0, hi=C):
            sl = rem(t, 2)
            rs = pl.ds(lo, hi - lo)
            ys = _output_transform([mbuf[sl, i, rs, :] for i in range(6)])
            bb = bias_ref[rs, :]
            for j in range(4):
                h = ys[j] + bb
                obuf[sl, j, rs, :] = (h + h * jnp.tanh(h)).astype(bf16)

        def xwait(c):
            xcopy(c, rem(c, R)).wait()

        def pre(t):
            if isinstance(t, int):
                if t + 1 < NI:
                    xwait(t + 1)
                if R - 1 <= t + R - 2 < NI:
                    xcopy(t + R - 2, (t + R - 2) % R).start()
            else:
                @pl.when(t + 1 < NI)
                def _():
                    xwait(t + 1)

                @pl.when(t + R - 2 < NI)
                def _():
                    xcopy(t + R - 2, rem(t + R - 2, R)).start()

        def stage(t, do):
            for i in range(6):
                if '3' in do:
                    for c in range(n3):
                        if (c * (6 - lag3)) // n3 + lag3 == i:
                            s3(t - 2, c * C // n3, (c + 1) * C // n3)
                if '2' in do:
                    s2(t - 1, i)
                if '1' in do:
                    for c in range(n1):
                        if (c * (6 - lag1)) // n1 + lag1 == i:
                            s1(t, c * C // n1, (c + 1) * C // n1)

        xwait(0)
        pre(0)
        s1(0)
        pre(1)
        stage(1, '12')

        def body(t, carry):
            pre(t)

            @pl.when(t >= 4)
            def _():
                ocopy(t - 4, rem(t, 2)).wait()

            stage(t, '123')
            ocopy(t - 2, rem(t, 2)).start()
            return carry

        lax.fori_loop(2, NI, body, None)
        ocopy(NI - 4, NI % 2).wait()
        stage(NI, '23')
        ocopy(NI - 2, NI % 2).start()
        ocopy(NI - 3, (NI - 3) % 2).wait()
        s3(NI - 1)
        ocopy(NI - 1, (NI - 1) % 2).start()
        ocopy(NI - 2, NI % 2).wait()
        ocopy(NI - 1, (NI - 1) % 2).wait()

    return kernel


@jax.jit
def pallas_standalone__batchnorm__sampling_kernel(
    x: jax.Array,
    w: jax.Array,
    mean: jax.Array,
    var: jax.Array,
    g: jax.Array,
    b: jax.Array,
):
    B, S, C = x.shape
    bn, R = 128, 4
    assert w.shape == (3, C, C) and S % 4 == 0 and B % bn == 0 and C % 96 == 0
    KT = -(-C // 128)
    f32, bf16, u32 = jnp.float32, jnp.bfloat16, jnp.uint32
    kernel = _make_kernel(S, C, B, bn, R, lag1=1, lag3=2, n1=6, n3=4)
    vec = pl.BlockSpec((C,), lambda: (0,))
    out = pl.pallas_call(
        kernel,
        grid=(),
        in_specs=[pl.BlockSpec(memory_space=pl.ANY),
                  pl.BlockSpec((3, C, C), lambda: (0, 0, 0)), vec, vec, vec, vec],
        out_specs=pl.BlockSpec(memory_space=pl.ANY),
        out_shape=jax.ShapeDtypeStruct((S, C, B), x.dtype),
        scratch_shapes=[
            pltpu.VMEM((R, 4, C, bn), bf16),
            pltpu.VMEM((2, 6, KT * 64, bn), u32),
            pltpu.VMEM((2, 6, C, bn), f32),
            pltpu.VMEM((2, 4, C, bn), bf16),
            pltpu.VMEM((6, KT, C // 2, 128), u32),
            pltpu.VMEM((C, 128), f32),
            pltpu.SemaphoreType.DMA((R,)),
            pltpu.SemaphoreType.DMA((2,)),
        ],
        compiler_params=pltpu.CompilerParams(vmem_limit_bytes=100 * 1024 * 1024),
    )(jnp.transpose(x, (1, 2, 0)), w, mean, var, g, b)
    return jnp.transpose(out, (2, 0, 1))
```

```python
import functools
import numpy as np
import jax
import jax.numpy as jnp
from jax import lax
import jax.experimental.pallas as pl
import jax.experimental.pallas.tpu as pltpu

_A = 1.5
_B = 2.0 / 3.0


def _filter_matrix():
    pts = [0.0, _A, -_A, _B, -_B]
    G = np.zeros((6, 3))
    for i, p in enumerate(pts):
        f = np.prod([p - q for k, q in enumerate(pts) if k != i])
        G[i] = [1.0 / f, p / f, p * p / f]
    G[5] = [0.0, 0.0, 1.0]
    return G


_G = _filter_matrix()


def _input_transform(d):
    d0, d1, d2, d3, d4, d5 = d
    a2, b2 = _A * _A, _B * _B
    a2d2 = a2 * d2
    b2d2 = b2 * d2
    eb = d4 - b2d2
    ea = d4 - a2d2
    ob = _A * (d3 - b2 * d1)
    oa = _B * (d3 - a2 * d1)
    t0 = (ea - b2d2) + d0
    t5 = (d5 + d1) - (a2 + b2) * d3
    return [t0, eb + ob, eb - ob, ea + oa, ea - oa, t5]


def _output_transform(m):
    m0, m1, m2, m3, m4, m5 = m
    s1 = m1 + m2
    d1 = m1 - m2
    s2 = m3 + m4
    d2 = m3 - m4
    y0 = m0 + s1 + s2
    y1 = _A * d1 + _B * d2
    y2 = (_A * _A) * s1 + (_B * _B) * s2
    y3 = (_A ** 3) * d1 + (_B ** 3) * d2 + m5
    return [y0, y1, y2, y3]


def _make_kernel(S, C, B, bn, R, pw):
    NG = S // 4
    NI = (B // bn) * NG
    KT = -(-C // 128)
    f32, bf16, u32 = jnp.float32, jnp.bfloat16, jnp.uint32

    def kernel(x_hbm, w_hbm, mean_ref, var_ref, g_ref, b_ref, o_hbm,
               xbuf, tbuf, mbuf, obuf, ubuf, bias_ref, w_ref, xsem, osem, wsem):
        def rem(t, m):
            return t % m if isinstance(t, int) else (t & (m - 1))

        def div(t, m):
            if isinstance(t, int):
                return t // m
            return lax.shift_right_logical(t, int(np.log2(m)))

        def window(ref, c):
            return ref.at[pl.ds(rem(c, NG) * 4, 4), :,
                          pl.ds(pl.multiple_of(div(c, NG) * bn, bn), bn)]

        def xcopy(c, slot):
            return pltpu.make_async_copy(window(x_hbm, c), xbuf.at[slot], xsem.at[slot])

        def ocopy(c, slot):
            return pltpu.make_async_copy(obuf.at[slot], window(o_hbm, c), osem.at[slot])

        wc = [pltpu.make_async_copy(w_hbm.at[k], w_ref.at[k], wsem.at[k]) for k in range(3)]
        wc[0].start()
        xcopy(0, 0).start()
        xcopy(1, 1).start()
        wc[2].start()
        wc[1].start()
        for c in range(2, R - 1):
            xcopy(c, c).start()

        def ld(r):
            return r[...].astype(f32)[None, :]

        sc = ld(g_ref) * (1.0 / jnp.sqrt(ld(var_ref) + 1e-5))
        bias = (ld(b_ref) - ld(mean_ref) * sc) * 0.5
        bias_ref[...] = jnp.broadcast_to(bias, (128, C)).T
        sch = sc * 0.5

        def make_u(i):
            for kk in range(KT):
                wdt = min(128, C - kk * 128)
                u = None
                for k in range(3):
                    if _G[i, k] != 0:
                        t = (w_ref[k, kk * 128:kk * 128 + wdt, :].astype(f32)
                             * (sch * float(_G[i, k])))
                        u = t if u is None else u + t
                v = u.astype(bf16)
                if wdt < 128:
                    v = jnp.concatenate([v, jnp.zeros((128 - wdt, C), bf16)], axis=0)
                ubuf[i, kk] = pltpu.bitcast(v.T, u32)

        for sl in range(2):
            for i in range(6):
                tbuf[sl, i, C // 2:, :] = jnp.zeros((KT * 64 - C // 2, bn), u32)

        def s1(t, lo=0, hi=C):
            g = rem(t, NG)
            sl = rem(t, 2)
            cm, cc, cp = rem(t + R - 1, R), rem(t, R), rem(t + 1, R)
            rs = pl.ds(lo, hi - lo)
            d0 = jnp.where(g > 0, xbuf[cm, 3, rs, :].astype(f32), 0.0)
            d5 = jnp.where(g < NG - 1, xbuf[cp, 0, rs, :].astype(f32), 0.0)
            d = [d0] + [xbuf[cc, j, rs, :].astype(f32) for j in range(4)] + [d5]
            tt = _input_transform(d)
            for i in range(6):
                tbuf[sl, i, pl.ds(lo // 2, (hi - lo) // 2), :] = pltpu.bitcast(
                    tt[i].astype(bf16), u32)

        def s2(t, i, between=()):
            sl = rem(t, 2)
            acc = None
            for kk in range(KT):
                lhs = pltpu.bitcast(ubuf[i, kk], bf16)
                rhs = pltpu.bitcast(tbuf[sl, i, kk * 64:(kk + 1) * 64, :], bf16)
                p = jnp.dot(lhs, rhs, preferred_element_type=f32)
                acc = p if acc is None else acc + p
            n = max(len(between), 1)
            for p in range(n):
                if between:
                    between[p]()
                mbuf[sl, i, p * C // n:(p + 1) * C // n, :] = acc[p * C // n:(p + 1) * C // n]

        def s3(t, lo=0, hi=C):
            sl = rem(t, 2)
            rs = pl.ds(lo, hi - lo)
            ys = _output_transform([mbuf[sl, i, rs, :] for i in range(6)])
            bb = bias_ref[rs, :]
            for j in range(4):
                h = ys[j] + bb
                obuf[sl, j, rs, :] = (h + h * jnp.tanh(h)).astype(bf16)

        def xwait(c):
            xcopy(c, rem(c, R)).wait()

        def pre(t):
            if isinstance(t, int):
                if t + 1 < NI:
                    xwait(t + 1)
                if R - 1 <= t + R - 2 < NI:
                    xcopy(t + R - 2, (t + R - 2) % R).start()
            else:
                @pl.when(t + 1 < NI)
                def _():
                    xwait(t + 1)

                @pl.when(t + R - 2 < NI)
                def _():
                    xcopy(t + R - 2, rem(t + R - 2, R)).start()

        def stage(t, with_input):
            tot = 4 * pw
            bounds = [16 * ((c * (C // 16)) // tot) for c in range(tot + 1)]
            for i in range(6):
                between = []
                if i >= 2:
                    for c in range((i - 2) * pw, (i - 1) * pw):
                        between.append(functools.partial(s3, t - 2, bounds[c], bounds[c + 1]))
                s2(t - 1, i, between)
            if with_input:
                s1(t)

        wc[0].wait()
        make_u(0)
        xwait(0)
        pre(0)
        s1(0)
        s2(0, 0)
        wc[2].wait()
        make_u(5)
        s2(0, 5)
        wc[1].wait()
        make_u(1)
        pre(1)
        for i in range(1, 5):
            s2(0, i)
            if i < 4:
                make_u(i + 1)
            s1(1, (i - 1) * C // 4, i * C // 4)

        def body(t, carry):
            pre(t)

            @pl.when(t >= 4)
            def _():
                ocopy(t - 4, rem(t, 2)).wait()

            stage(t, True)
            ocopy(t - 2, rem(t, 2)).start()
            return carry

        lax.fori_loop(2, NI, body, None)
        ocopy(NI - 4, NI % 2).wait()
        stage(NI, False)
        ocopy(NI - 2, NI % 2).start()
        ocopy(NI - 3, (NI - 3) % 2).wait()
        s3(NI - 1)
        ocopy(NI - 1, (NI - 1) % 2).start()
        ocopy(NI - 2, NI % 2).wait()
        ocopy(NI - 1, (NI - 1) % 2).wait()

    return kernel


@jax.jit
def pallas_standalone__batchnorm__sampling_kernel(
    x: jax.Array,
    w: jax.Array,
    mean: jax.Array,
    var: jax.Array,
    g: jax.Array,
    b: jax.Array,
):
    B, S, C = x.shape
    bn, R = 128, 4
    assert w.shape == (3, C, C) and S % 4 == 0 and B % bn == 0 and C % 64 == 0
    KT = -(-C // 128)
    f32, bf16, u32 = jnp.float32, jnp.bfloat16, jnp.uint32
    kernel = _make_kernel(S, C, B, bn, R, pw=4)
    vec = pl.BlockSpec((C,), lambda: (0,))
    out = pl.pallas_call(
        kernel,
        grid=(),
        in_specs=[pl.BlockSpec(memory_space=pl.ANY),
                  pl.BlockSpec(memory_space=pl.ANY), vec, vec, vec, vec],
        out_specs=pl.BlockSpec(memory_space=pl.ANY),
        out_shape=jax.ShapeDtypeStruct((S, C, B), x.dtype),
        scratch_shapes=[
            pltpu.VMEM((R, 4, C, bn), bf16),
            pltpu.VMEM((2, 6, KT * 64, bn), u32),
            pltpu.VMEM((2, 6, C, bn), f32),
            pltpu.VMEM((2, 4, C, bn), bf16),
            pltpu.VMEM((6, KT, C // 2, 128), u32),
            pltpu.VMEM((C, 128), f32),
            pltpu.VMEM((3, C, C), bf16),
            pltpu.SemaphoreType.DMA((R,)),
            pltpu.SemaphoreType.DMA((2,)),
            pltpu.SemaphoreType.DMA((3,)),
        ],
        compiler_params=pltpu.CompilerParams(vmem_limit_bytes=100 * 1024 * 1024),
    )(jnp.transpose(x, (1, 2, 0)), w, mean, var, g, b)
    return jnp.transpose(out, (2, 0, 1))
```
